```python
import os as _os
_os.environ.setdefault("JAX_PLATFORMS", "cpu")
import jax
import jax.numpy as jnp

def _softmax(x, axis=-1):
    return jax.nn.softmax(x, axis=axis)
def _gelu(x):
    return jax.nn.gelu(x, approximate=True)
def _silu(x):
    return jax.nn.silu(x)
def _sigmoid(x):
    return jax.nn.sigmoid(x)
def _layernorm(x, axis=-1, eps=1e-5):
    m = jnp.mean(x, axis=axis, keepdims=True)
    v = jnp.var(x, axis=axis, keepdims=True)
    return (x - m) / jnp.sqrt(v + eps)
def _scatter_add(tgt, idx, src, axis=0):
    return tgt.at[idx].add(src)
def _segment_sum(src, seg, n):
    return jax.ops.segment_sum(src, seg, n)
class _Rng:
    def __init__(self, key):
        self._k = key
    def _next(self):
        self._k, sub = jax.random.split(self._k)
        return sub
    def normal(self, shape):
        return jax.random.normal(self._next(), shape, dtype=jnp.bfloat16)
    def randint(self, lo, hi, shape):
        return jax.random.randint(self._next(), shape, lo, hi, dtype=jnp.int32)
    def uniform(self, shape, lo=0.0, hi=1.0):
        return jax.random.uniform(self._next(), shape, jnp.bfloat16, lo, hi)
    def permutation(self, n):
        return jax.random.permutation(self._next(), n)


kernel_name = 'concat_heads__ssm_conv_h3__sliding_block__prompt'

def setup_inputs():
    _rng = _Rng(jax.random.key(int.from_bytes(__import__("os").urandom(4), "little")))
    _w = (lambda a: (lambda t: t.astype(jnp.bfloat16) if jnp.issubdtype(t.dtype, jnp.floating) else t)(jnp.asarray(a)))
    def _A_setup():
        B, S, D = 1, 2048, 512
        ks = 4
        return {
            "q": _w((lambda *s: _rng.normal(s) * 0.05)(B, S, D)),
            "k": _w((lambda *s: _rng.normal(s) * 0.2)(B, S, D)),
            "v": _w((lambda *s: _rng.normal(s) * 0.2)(B, S, D)),
            "shift_k": _w((lambda *s: _rng.normal(s) * 0.2)(D, ks) * 0.5),
            "ssm_k": _w((lambda *s: _rng.normal(s) * 0.2)(D, S) * (1.0 / S ** 0.5)),
            "ssm_D": _w((lambda *s: _rng.normal(s) * 0.2)(D)),
        }
    _A_in = _A_setup()

    def _B_setup():
        B, S, D = 1, 2048, 512
        return {
            "x": _w((lambda *s: _rng.normal(s) * 0.2)(B, S, D)),
            "wqkv": _w((lambda *s: _rng.normal(s) * 0.2)(D, 3 * D)),
            "wo": _w((lambda *s: _rng.normal(s) * 0.05)(D, D)),
        }
    _B_in = _B_setup()

    return {
        "A_q": _A_in["q"],
        "A_k": _A_in["k"],
        "A_v": _A_in["v"],
        "A_shift_k": _A_in["shift_k"],
        "A_ssm_k": _A_in["ssm_k"],
        "A_ssm_D": _A_in["ssm_D"],
        "B_x": _B_in["x"],
        "B_wqkv": _B_in["wqkv"],
        "B_wo": _B_in["wo"],
    }

def reference(A_q, A_k, A_v, A_shift_k, A_ssm_k, A_ssm_D, B_x, B_wqkv, B_wo):
    def _A_ref(q, k, v, shift_k, ssm_k, ssm_D):
        B, S, D = q.shape
        ks = shift_k.shape[-1]
        k_pad = jnp.pad(k, ((0, 0), (ks - 1, 0), (0, 0)))
        k_shift = jnp.zeros_like(k)
        for t in range(ks):
            k_shift = k_shift + k_pad[:, t:t + S, :] * shift_k[:, ks - 1 - t][None, None, :]
        kv = k_shift * v
        L = 2 * S
        kv_pad = jnp.pad(kv, ((0, 0), (0, S), (0, 0)))
        kf_pad = jnp.pad(ssm_k, ((0, 0), (0, S)))
        kv_f = (lambda x, axes=(-2,-1): jnp.fft.rfft2(x.astype(jnp.float32), axes=axes))(kv_pad[:, None, :, :], axes=(1, 2))
        kf_f = (lambda x, axes=(-2,-1): jnp.fft.rfft2(x.astype(jnp.float32), axes=axes))(kf_pad[:, None, :], axes=(1, 2))
        kf_f = (lambda x, *d: x.transpose(*d))(kf_f, 1, 2, 0)
        y_f = kv_f * kf_f[None, :, :, :]
        y = (lambda x, s, axes=(-2,-1): jnp.fft.irfft2(x, s=s, axes=axes).astype(jnp.bfloat16))(y_f, (1, L), axes=(1, 2))[:, 0, :S, :]
        y = y + kv * ssm_D[None, None, :]
        return q * y

    def _B_ref(x, wqkv, wo):
        B, S, D = x.shape
        H = 32; Dh = D // H; W = 256
        qkv = (lambda x, *d: x.transpose(*d))((x @ wqkv).reshape(B, S, 3, H, Dh), 2, 0, 3, 1, 4)
        q, k, v = qkv[0], qkv[1], qkv[2]
        scores = jnp.einsum("bhqd,bhkd->bhqk", q, k) * (Dh ** -0.5)
        idx = jnp.arange(S)
        mask = (idx[:, None] - idx[None, :] >= 0) & (idx[:, None] - idx[None, :] < W)
        scores = jnp.where(mask[None, None], scores, -1e9)
        p = _softmax(scores, axis=-1)
        o = jnp.einsum("bhqk,bhkd->bhqd", p, v)
        return (lambda x, *d: x.transpose(*d))(o, 0, 2, 1, 3).reshape(B, S, D) @ wo

    a = _A_ref(A_q, A_k, A_v, A_shift_k, A_ssm_k, A_ssm_D)
    b = _B_ref(B_x, B_wqkv, B_wo)
    return jnp.concatenate([a, b], axis=-1)
```

```python
import functools
import numpy as np
import jax
import jax.numpy as jnp
from jax import lax
from jax.experimental import pallas as pl
from jax.experimental.pallas import tpu as pltpu

S, D, H, DH, WIN = 2048, 512, 32, 16, 256
T = 128
NB = S // T
PADK = 2 * T
NEG = -1e30
QSCALE = float(DH ** -0.5 * np.log2(np.e))
TOKS = 48


def _dft_consts():
    n = np.arange(T, dtype=np.float64)
    f = np.arange(T, dtype=np.float64)
    th = 2.0 * np.pi * (f[:, None] + 0.5) * n[None, :] / (2 * T)
    fwd = np.concatenate([np.cos(th), -np.sin(th)], axis=0)
    inv = np.concatenate([np.cos(th).T, -np.sin(th).T], axis=1) / T
    return fwd.astype(np.float32), inv.astype(np.float32)


UROT = (0, 2, 0)
HROT = (1, 1, 3)


def _st(ref, i, comp, val, rot):
    for c in range(4):
        cc = (c + rot[comp]) % 4
        ref[i, comp, :, cc * 128:(cc + 1) * 128] = val[:, c * 128:(c + 1) * 128]


def _ld(ref, i, comp, c, rot):
    cc = (c + rot[comp]) % 4
    return ref[i, comp, :, cc * 128:(cc + 1) * 128]


def _kernel(q_ref, k_ref, v_ref, sk_ref, hk_ref, dd_ref, x_ref, wqkv_ref, wo_ref, f_ref, g_ref,
            o_ref,
            kc, vtc, ot, sb0, sb1, mb0, mb1, us, hs, hprev, khalo):
    t = pl.program_id(0)
    base = pl.multiple_of(t * T, T)
    f32, bf16 = jnp.float32, jnp.bfloat16

    @pl.when(t == 0)
    def _init():
        kc[0:PADK, :] = jnp.zeros((PADK, D), bf16)
        vtc[:, 0:PADK] = jnp.zeros((D, PADK), bf16)
        us[NB] = jnp.zeros((3, T, D), f32)
        hprev[...] = jnp.zeros((2 * T, D), f32)
        khalo[...] = jnp.zeros((8, D), f32)

    qkv = jnp.dot(x_ref[0], wqkv_ref[...], preferred_element_type=f32)
    qn = (qkv[:, 0:D] * QSCALE).astype(bf16)
    kc[pl.ds(base + PADK, T), :] = qkv[:, D:2 * D].astype(bf16)
    vtc[:, pl.ds(base + PADK, T)] = qkv[:, 2 * D:3 * D].T.astype(bf16)

    kf = k_ref[0].astype(f32)
    kext = jnp.concatenate([khalo[...], kf], axis=0)
    khalo[...] = kf[T - 8:T, :]
    skw = sk_ref[...].astype(f32)
    ksh = kf * skw[0:1, :]
    for j in range(1, 4):
        ksh = ksh + kext[8 - j:8 - j + T, :] * skw[j:j + 1, :]
    kv_b = (ksh * v_ref[0].astype(f32)).astype(bf16)
    uf = jnp.dot(f_ref[...], kv_b, preferred_element_type=f32)
    _st(us, t, 0, uf[0:T], UROT)
    _st(us, t, 1, uf[T:2 * T], UROT)
    _st(us, t, 2, uf[0:T] + uf[T:2 * T], UROT)
    hf = lax.dot_general(f_ref[...], hk_ref[...], (((1,), (1,)), ((), ())),
                         preferred_element_type=f32)
    sgn = (1 - 2 * (lax.broadcasted_iota(jnp.int32, (T, D), 0) & 1)).astype(f32)
    h2r = hf[0:T] - sgn * hprev[T:2 * T, :]
    h2i = hf[T:2 * T] + sgn * hprev[0:T, :]
    hprev[...] = hf
    _st(hs, t, 0, h2r, HROT)
    _st(hs, t, 1, h2i - h2r, HROT)
    _st(hs, t, 2, h2r + h2i, HROT)

    ki = lax.broadcasted_iota(jnp.int32, (T, T), 0)
    qi = lax.broadcasted_iota(jnp.int32, (T, T), 1)
    tri = ki <= qi
    lane_head = qi // DH
    bias_old = jnp.where(t >= 2, 0.0, NEG).astype(f32)
    bias_mid = jnp.where(t >= 1, 0.0, NEG).astype(f32)
    sb = [sb0, sb1]
    mb = [mb0, mb1]

    def stage_a(j):
        g = j // 2
        qg = qn[:, g * 128:(g + 1) * 128]
        wt = jnp.concatenate(
            [jnp.where(lane_head == (j % 2) * 4 + u, qg, jnp.zeros_like(qg)) for u in range(4)], axis=0)
        pieces = []
        for r in range(T // 16):
            pieces.append(kc[pl.ds(base + r * 16, 16), g * 128:(g + 1) * 128])
            pieces.append(kc[pl.ds(base + 2 * T + r * 16, 16), g * 128:(g + 1) * 128])
            if r % 2 == 1:
                pieces.append(kc[pl.ds(base + T + (r - 1) * 16, 32), g * 128:(g + 1) * 128])
        lhs = jnp.concatenate(pieces, axis=0)
        s = lax.dot_general(lhs, wt, (((1,), (1,)), ((), ())), preferred_element_type=f32)
        toks = [s[u * TOKS:u * TOKS + 1, u * 128:(u + 1) * 128] for u in range(4)]
        for u in range(4):
            su = s[:, u * 128:(u + 1) * 128]
            mm = None
            for p in range(T // 32):
                b0 = p * 96
                for r in range(2):
                    off = p * 32 + r * 16
                    old = su[b0 + r * 32:b0 + r * 32 + 16] + bias_old
                    new = su[b0 + r * 32 + 16:b0 + r * 32 + 32]
                    comb = jnp.where(tri[off:off + 16], new, old)
                    sb[j % 2][u, off:off + 16, :] = comb
                    c8 = jnp.maximum(comb[:8], comb[8:])
                    mm = c8 if mm is None else jnp.maximum(mm, c8)
                mid = su[b0 + 64:b0 + 96] + bias_mid
                sb[j % 2][u, T + p * 32:T + (p + 1) * 32, :] = mid
                mm = jnp.maximum(mm, mid.reshape(4, 8, T).max(axis=0))
            mb[j % 2][u] = jnp.broadcast_to(jnp.max(mm, axis=0, keepdims=True), (8, T))
        return toks

    def stage_b(j, toks):
        g = j // 2
        for u in range(4):
            h = g * 8 + (j % 2) * 4 + u
            m = mb[j % 2][u][0:1, :]
            if toks is not None:
                m = jnp.maximum(m, jnp.minimum(m, toks[u]))
            p = jnp.exp2(sb[j % 2][u] - m)
            l = jnp.sum(p, axis=0, keepdims=True)
            pc = p[:T]
            pm = p[T:]
            p_new = jnp.where(tri, pc, 0.0).astype(bf16)
            p_old = jnp.where(tri, 0.0, pc).astype(bf16)
            vh = vtc[h * 16:(h + 1) * 16, pl.ds(base, 3 * T)]
            r = jnp.dot(vh[:, 0:T], p_old, preferred_element_type=f32)
            r += jnp.dot(vh[:, T:2 * T], pm.astype(bf16), preferred_element_type=f32)
            r += jnp.dot(vh[:, 2 * T:], p_new, preferred_element_type=f32)
            ot[h * 16:(h + 1) * 16, :] = r * (1.0 / l)

    toks = stage_a(0)
    for j in range(8):
        toks = stage_a(j + 1) if j + 1 < 8 else None
        stage_b(j, toks)

    cols = []
    for c in range(4):
        k1 = jnp.zeros((T, 128), f32)
        k2 = jnp.zeros((T, 128), f32)
        k3 = jnp.zeros((T, 128), f32)
        for a in range(NB):
            ua = jnp.where(a <= t, a, NB)
            hd = jnp.maximum(t - a, 0)
            k1 = k1 + _ld(hs, hd, 0, c, HROT) * _ld(us, ua, 2, c, UROT)
            k2 = k2 + _ld(us, ua, 0, c, UROT) * _ld(hs, hd, 1, c, HROT)
            k3 = k3 + _ld(us, ua, 1, c, UROT) * _ld(hs, hd, 2, c, HROT)
        cols.append(jnp.concatenate([k1 - k3, k1 + k2], axis=0).astype(bf16))
    wsp = jnp.concatenate(cols, axis=1)
    y = jnp.dot(g_ref[...], wsp, preferred_element_type=f32)
    y = y + kv_b.astype(f32) * dd_ref[...].astype(f32)
    o_ref[0, :, 0:D] = (q_ref[0].astype(f32) * y).astype(o_ref.dtype)

    on = ot[...].T.astype(bf16)
    o_ref[0, :, D:2 * D] = jnp.dot(on, wo_ref[...], preferred_element_type=f32).astype(o_ref.dtype)


@jax.jit
def pallas_concat_heads__ssm_conv_h3__sliding_block__prompt_kernel(A_q, A_k, A_v, A_shift_k, A_ssm_k, A_ssm_D, B_x, B_wqkv, B_wo):
    fwd, inv = _dft_consts()
    fwd = jnp.asarray(fwd, jnp.bfloat16)
    inv = jnp.asarray(inv, jnp.bfloat16)
    row = lambda t: (0, t, 0)
    const = lambda t: (0, 0)
    f32, bf16 = jnp.float32, jnp.bfloat16
    return pl.pallas_call(
        _kernel,
        grid=(NB,),
        in_specs=[
            pl.BlockSpec((1, T, D), row), pl.BlockSpec((1, T, D), row), pl.BlockSpec((1, T, D), row),
            pl.BlockSpec((4, D), const),
            pl.BlockSpec((D, T), lambda t: (0, t)),
            pl.BlockSpec((1, D), const),
            pl.BlockSpec((1, T, D), row),
            pl.BlockSpec((D, 3 * D), const),
            pl.BlockSpec((D, D), const),
            pl.BlockSpec((2 * T, T), const),
            pl.BlockSpec((T, 2 * T), const),
        ],
        out_specs=pl.BlockSpec((1, T, 2 * D), row),
        out_shape=jax.ShapeDtypeStruct((1, S, 2 * D), bf16),
        scratch_shapes=[
            pltpu.VMEM((S + PADK, D), bf16),
            pltpu.VMEM((D, S + PADK), bf16),
            pltpu.VMEM((D, T), f32),
            pltpu.VMEM((4, 2 * T, T), f32), pltpu.VMEM((4, 2 * T, T), f32),
            pltpu.VMEM((4, 8, T), f32), pltpu.VMEM((4, 8, T), f32),
            pltpu.VMEM((NB + 1, 3, T, D), f32),
            pltpu.VMEM((NB, 3, T, D), f32),
            pltpu.VMEM((2 * T, D), f32),
            pltpu.VMEM((8, D), f32),
        ],
        compiler_params=pltpu.CompilerParams(dimension_semantics=("arbitrary",),
                                             vmem_limit_bytes=100 * 1024 * 1024),
    )(A_q, A_k, A_v, A_shift_k.T, A_ssm_k, A_ssm_D.reshape(1, D), B_x, B_wqkv, B_wo, fwd, inv)
```

```python
import functools
import numpy as np
import jax
import jax.numpy as jnp
from jax import lax
from jax.experimental import pallas as pl
from jax.experimental.pallas import tpu as pltpu

S, D, H, DH, WIN = 2048, 512, 32, 16, 256
T = 128
HT = T // 2
NB = S // T
QSCALE = float(DH ** -0.5 * np.log2(np.e))
UROT = (0, 2, 0)
HROT = (1, 1, 3)
CROWS = 16
MERGE = 13
LA = 4
NEG = -1e30
NDEF = 2
DSTR = 2
KVSTR = 8
BPOS = 2
BSTR = 3
ORDER = "inv K0 Q0 O2 B6 V0 K1 B7 P0 A0 Q1 O3 A1 V1 K2 B0 P1 A2 Q2 V2 B1 A3 K3 Q3 B2 P2 A4 V3 O0 B3 A5 Hf B4 P3 A6 O1 Uf B5 A7"
ORDER2 = "inv K0 Q0 O2 B6 V0 K1 B7 P0 A0 Q1 O3 A1 V1 K2 B0 P1 A2 Q2 V2 B1 A3 K3 Q3 B2 P2 A4 V3 O0 B3 A5 P3 O1 B4 A6 Uf B5 A7"
ORDER1 = "w0 K0 Q0 V0 w1 K1 Q1 P0 A0 V1 A1 w2 K2 Q2 B0 P1 A2 V2 B1 A3 w3 K3 Q3 B2 P2 A4 V3 w4 O0 B3 A5 Hf B4 P3 A6 O1 Uf B5 A7"
LAG = 2
PRUNG = [0, 32, 64, 96]
KVPOS = 12
VARIANTS = [(0, 0), (1, 1), (2, 2), (3, 3), (4, 8), (9, 11), (12, 12), (13, 13), (14, 14), (15, 15), (16, 16), (17, 17)]
f32, bf16, u32 = jnp.float32, jnp.bfloat16, jnp.uint32


def _pack_np(a):
    u = np.ascontiguousarray(a, np.float32).view(np.uint32).astype(np.uint64)
    b = ((u + 0x7FFF + ((u >> 16) & 1)) >> 16).astype(np.uint32)
    return b[0::2] | (b[1::2] << 16)


def _dft_consts():
    n = np.arange(T, dtype=np.float64)
    f = np.arange(T, dtype=np.float64)
    th = 2.0 * np.pi * (f[:, None] + 0.5) * n[None, :] / (2 * T)
    fwd = np.stack([np.cos(th).reshape(T // 16, 16, T), -np.sin(th).reshape(T // 16, 16, T)], axis=1)
    fwd = fwd.reshape(2 * T, T)
    inv = np.concatenate([np.cos(th).T, -np.sin(th).T], axis=1) / T
    return fwd.astype(np.float32), inv.astype(np.float32)


def _st(ref, i, comp, val, rot):
    for c in range(4):
        cc = (c + rot[comp]) % 4
        ref[i, comp, :, cc * 128:(cc + 1) * 128] = val[:, c * 128:(c + 1) * 128]


def _ld(ref, i, comp, r0, r1, c, rot):
    cc = (c + rot[comp]) % 4
    return ref[i, comp, r0:r1, cc * 128:(cc + 1) * 128]


def _after(val, tok):
    return jnp.where(tok > jnp.inf, tok.astype(val.dtype), val)


def _fold(x):
    x = x.reshape(x.shape[0] // 8, 8, x.shape[1]).max(axis=0)
    out = x[:, 0:128]
    for c in range(1, x.shape[1] // 128):
        out = jnp.maximum(out, x[:, c * 128:(c + 1) * 128])
    return out


def _prow(start, size):
    if isinstance(start, int):
        return slice(start // 2, (start + size) // 2)
    return pl.ds(pl.multiple_of(start // 2, 8), size // 2)


def _lanes(start):
    if isinstance(start, int):
        return slice(start, start + T)
    return pl.ds(pl.multiple_of(start, T), T)


def _unp(x):
    return pltpu.bitcast(x, bf16)


def _pk(x):
    return pltpu.bitcast(x.astype(bf16), u32)


def _step(lo, hi, s, q_hbm, k_hbm, v_hbm, sk_hbm, hk_hbm, dd_hbm, x_hbm, wqkv_hbm, wo_hbm, f_hbm, g_hbm,
          o_hbm,
          qb, kb, vb, xb, hkb, sk_ref, dd_ref, f_ref, g_ref, obuf, isem, osem,
          wstage, wq, wo, sems, xs, kc0, kc1, kc2, kc3, vt0, vt1, vt2, vt3, sb0, sb1, mb0, mb1, pk, us, hs,
          yprev, khalo, wsp, qts, kvs, ots, accs):
    do_front, do_main, do_fin = lo < NB, 1 <= lo <= NB, lo >= 2
    t = s - 1
    base = t * T
    ki = lax.broadcasted_iota(jnp.int32, (T, T), 0)
    qi = lax.broadcasted_iota(jnp.int32, (T, T), 1)
    tris = (ki <= qi, ki <= (qi ^ HT))
    sb = [sb0, sb1]
    kc = [kc0, kc1, kc2, kc3]
    vtc = [vt0, vt1, vt2, vt3]
    mb = [mb0, mb1]

    def wcopy(i):
        c0 = (i % 3) * D + (i // 3) * 128
        if i < 12:
            return pltpu.make_async_copy(wqkv_hbm.at[:, c0:c0 + 128], wstage.at[:, c0:c0 + 128], sems.at[i])
        return pltpu.make_async_copy(wo_hbm, wstage.at[:, 3 * D:4 * D], sems.at[12])

    def repack(i, tok):
        c0 = i * 128
        words = pltpu.bitcast(wstage[:, c0:c0 + 128], u32)
        if i < 12:
            wq[:, c0:c0 + 128] = words
        else:
            wo[:, c0 - 3 * D:c0 - 3 * D + 128] = words
        return None

    def rowblk(b):
        return slice(b * T, (b + 1) * T) if isinstance(b, int) else pl.ds(pl.multiple_of(b * T, T), T)

    def cin(i, b, rest=False):
        if i == 4:
            if isinstance(b, int) and b < LA:
                cols = slice(2 * b * T, (2 * b + 2) * T)
            else:
                cols = rowblk(b + LA)
            return pltpu.make_async_copy(hk_hbm.at[:, cols], hkb.at[:, cols], isem.at[4])
        src_, dst = ((k_hbm, kb), (v_hbm, vb), (x_hbm, xb), (q_hbm, qb))[i]
        rows = slice(b * T, S) if rest else rowblk(b)
        return pltpu.make_async_copy(src_.at[0, rows, :], dst.at[rows, :], isem.at[i])

    def csmall(i):
        src_, dst = ((f_hbm, f_ref), (sk_hbm, sk_ref), (g_hbm, g_ref), (dd_hbm, dd_ref))[i]
        return pltpu.make_async_copy(src_, dst, isem.at[5 + i])

    def cout(step):
        return pltpu.make_async_copy(obuf.at[rowblk(step - 2), :], o_hbm.at[0, rowblk(step - 2), :], osem.at[0])

    FRONT = (4, 0, 1)
    def wstart(g):
        for i in (1, 0, 2):
            wcopy(3 * g + i).start()

    if lo == 0:
        csmall(0).start()
        for i in FRONT:
            cin(i, 0).start()
        csmall(1).start()
        us[0:LA] = jnp.zeros((LA, 3, T, D), f32)
        cin(2, 0).start()
        wstart(0)
        csmall(0).wait()
        csmall(1).wait()
        for i in FRONT:
            cin(i, 0).wait()
        wstart(1)
    elif lo == 1:
        cin(2, 0).wait()
        cin(2, 1).start()
        cin(3, 0).start()
    else:
        if lo == 2:
            csmall(2).wait()
            csmall(3).wait()
        def guarded(last, fn):
            if hi <= last:
                fn()
            elif lo <= last:
                pl.when(s <= last)(fn)

        if lo <= MERGE:
            rest = lo == MERGE
            guarded(NB - 1, lambda: [cin(i, s, rest).wait() for i in (0, 1)] and None)
            guarded(NB - 1 - LA, lambda: cin(4, s).wait())
            cin(2, s - 1, rest).wait()
            cin(3, s - 2, rest).wait()
        if lo < MERGE:
            rest = lo == MERGE - 1
            assert not rest or lo == hi
            guarded(NB - 2, lambda: [cin(i, s + 1, rest).start() for i in (0, 1)] and None)
            guarded(NB - 2 - LA, lambda: cin(4, s + 1).start())
            cin(2, s, rest).start()
            cin(3, s - 1, rest).start()

    k_blk = kb.at[rowblk(jnp.minimum(s, NB - 1) if not isinstance(s, int) else min(s, NB - 1)), :]
    v_blk = vb.at[rowblk(jnp.minimum(s, NB - 1) if not isinstance(s, int) else min(s, NB - 1)), :]
    o_ref = obuf.at[rowblk(s - 2), :] if do_fin else None

    pieces, pend = [], []

    def rung(val):
        out = val
        if len(pend) >= LAG:
            tk = pend.pop(0)
            if tk is not None:
                out = _after(val, tk)
        pend.append(pieces.pop(0)(val) if pieces else None)
        return out

    def rungs(val, rows):
        parts, prev = [], 0
        for r in rows:
            if r > prev:
                parts.append(val[prev:r])
            row = val[r:r + 8]
            if row.shape[1] > 128:
                row = jnp.concatenate([rung(row[:, 0:128]), row[:, 128:]], axis=1)
            else:
                row = rung(row)
            parts.append(row)
            prev = r + 8
        parts.append(val[prev:])
        return jnp.concatenate(parts, axis=0)

    def b_exp(j, u, tok, has_mid):
        m = mb[j % 2][u][0:1, :]
        if tok is not None:
            m = _after(m, tok)
        p = jnp.exp2(sb[j % 2][u, 0:(2 * T if has_mid else T), :] - m)
        n = p.shape[0] // 32
        part = p.reshape(n, 4, 8, T).sum(axis=0)
        l8 = (part[0] + part[1]) + (part[2] + part[3])
        return p, jnp.sum(l8, axis=0, keepdims=True), l8

    def b_v(j, u, b0, has_old, has_mid):
        h = j * 4 + u
        return [_unp(vtc[h // 8][_prow((h % 8) * 16, 16), _lanes(b0 - i * T)])
                for i in range(1 + has_mid + has_old)]

    def b_pv(j, u, p, l, vs):
        h = j * 4 + u
        tri = tris[u % 2]
        pc = p[:T]
        r = jnp.dot(vs[0], jnp.where(tri, pc, 0.0).astype(bf16), preferred_element_type=f32)
        if len(vs) > 1:
            r += jnp.dot(vs[1], p[T:].astype(bf16), preferred_element_type=f32)
        if len(vs) > 2:
            r += jnp.dot(vs[2], jnp.where(tri, 0.0, pc).astype(bf16), preferred_element_type=f32)
        r = r * (1.0 / l)
        if u % 2:
            r = pltpu.roll(r, HT, 1)
        ots[h * 16:(h + 1) * 16, :] = r

    def outproj(g):
        og = ots[g * 128:(g + 1) * 128, :].T.astype(bf16)
        w = wstage[g * 128:(g + 1) * 128, 3 * D:4 * D] if lo == 1 else _unp(wo[_prow(g * 128, 128), :])
        part = jnp.dot(og, w, preferred_element_type=f32)
        part = rungs(part, [0, 64])
        if g == 0:
            accs[...] = part
        elif g < 3:
            accs[...] += part
        else:
            o_ref[:, D:2 * D] = (accs[...] + part).astype(o_ref.dtype)

    cks = []
    COMPS = ((hs, 0, HROT, us, 2, UROT), (us, 0, UROT, hs, 1, HROT), (us, 1, UROT, hs, 2, HROT))

    def conv_out(blk, k1, k2, k3):
        c, rb = blk % 4, blk // 4
        r0, r1 = rb * CROWS, (rb + 1) * CROWS
        cl = slice(c * 128, (c + 1) * 128)
        yr, yi = k1 - k3, k1 + k2
        wr, wi = yr, yi
        if lo > 1:
            sgn = (1 - 2 * (lax.broadcasted_iota(jnp.int32, (CROWS, 128), 0) & 1)).astype(f32)
            wr = yr - sgn * yprev[T + r0:T + r1, cl]
            wi = yi + sgn * yprev[r0:r1, cl]
        yprev[r0:r1, cl] = yr
        yprev[T + r0:T + r1, cl] = yi
        wsp[_prow(r0, CROWS), cl] = _pk(wr)
        wsp[_prow(T + r0, CROWS), cl] = _pk(wi)

    pairs = [(t + (LA - d), d) for d in range(hi)]

    def conv_chain(i, tok):
        blk, comp = i // 3, i % 3
        c, rb = blk % 4, blk // 4
        r0, r1 = rb * CROWS, (rb + 1) * CROWS
        if tok is not None:
            tok = jnp.concatenate([tok] * (CROWS // 8), axis=0)
        if lo != hi:
            n = len(pairs)
            acc = cks.pop() if comp else None
            cuts = [0, (n + 2) // 3, (2 * n + 2) // 3, n]
            for (iu, ih) in pairs[cuts[comp]:cuts[comp + 1]]:
                ur = _ld(us, iu, 0, r0, r1, c, UROT)
                ui = _ld(us, iu, 1, r0, r1, c, UROT)
                if tok is not None:
                    ur = _after(ur, tok)
                    tok = None
                ps = (_ld(hs, ih, 0, r0, r1, c, HROT) * (ur + ui), ur * _ld(hs, ih, 1, r0, r1, c, HROT),
                      ui * _ld(hs, ih, 2, r0, r1, c, HROT))
                acc = ps if acc is None else tuple(a + p for a, p in zip(acc, ps))
            if comp == 2:
                conv_out(blk, *acc)
            else:
                cks.append(acc)
            return _fold(jnp.maximum(jnp.maximum(acc[0], acc[1]), acc[2]))
        ra, ca, rota, rb_, cb, rotb = COMPS[comp]
        acc = None
        for (iu, ih) in pairs:
            ia = ih if ra is hs else iu
            ib = ih if rb_ is hs else iu
            p = _ld(ra, ia, ca, r0, r1, c, rota) * _ld(rb_, ib, cb, r0, r1, c, rotb)
            if acc is None:
                acc = p if tok is None else _after(p, tok)
            else:
                acc = acc + p
        cks.append(acc)
        if comp == 2:
            conv_out(blk, *cks)
            del cks[:]
        return _fold(acc)

    def kv_piece(i, tok):
        rb, lh = i // 2, i % 2
        ln = slice(lh * 256, (lh + 1) * 256)
        cur = k_blk[rb * 32:(rb + 1) * 32, ln].astype(f32)
        if tok is not None:
            cur = jnp.concatenate(
                [jnp.concatenate([_after(cur[0:8, 0:128], tok), cur[0:8, 128:]], axis=1), cur[8:]], axis=0)
        if rb > 0:
            prev8 = k_blk[rb * 32 - 16:rb * 32, ln].astype(f32)[8:16]
        elif lo == 0:
            prev8 = jnp.zeros((8, 256), f32)
        else:
            prev8 = khalo[:, ln]
        ext = jnp.concatenate([prev8, cur], axis=0)
        skw = sk_ref[:, ln].astype(f32)
        ksh = cur * skw[0:1, :]
        for j in range(1, 4):
            ksh = ksh + ext[8 - j:40 - j, :] * skw[j:j + 1, :]
        kv = ksh * v_blk[rb * 32:(rb + 1) * 32, ln].astype(f32)
        kvs[s % 4, _prow(rb * 32, 32), ln] = _pk(kv)
        if rb == 3:
            khalo[:, ln] = cur[24:32]
        return _fold(kv)

    def split(x):
        x = x.reshape(T // 16, 2, 16, D)
        return x[:, 0].reshape(T, D), x[:, 1].reshape(T, D)

    def front_h(c):
        hf = lax.dot_general(_unp(f_ref[...]), hkb[:, rowblk(c)], (((1,), (1,)), ((), ())),
                             preferred_element_type=f32)
        hr, hi_ = split(rungs(hf, [0, 64, 128, 192]))
        _st(hs, c, 0, hr, HROT)
        _st(hs, c, 1, hi_ - hr, HROT)
        _st(hs, c, 2, hr + hi_, HROT)

    def front_hs():
        if lo < LA:
            return [2 * lo, 2 * lo + 1]
        if lo + LA >= NB:
            return []
        return [s + LA if hi + LA < NB else jnp.minimum(s + LA, NB - 1)]

    def front_u():
        for pc in [pc for pc in pieces if pc.func is kv_piece]:
            pieces.remove(pc)
            pc(None)
        uf = jnp.dot(_unp(f_ref[...]), _unp(kvs[s % 4]), preferred_element_type=f32)
        ur, ui = split(rungs(uf, [0, 64, 128, 192]))
        _st(us, s + LA, 0, ur, UROT)
        _st(us, s + LA, 1, ui, UROT)
        _st(us, s + LA, 2, ur + ui, UROT)

    def conv_finish():
        y = jnp.dot(_unp(g_ref[...]), _unp(wsp[...]), preferred_element_type=f32)
        y = rungs(y, PRUNG)
        y = y + _unp(kvs[(s - 2) % 4]).astype(f32) * dd_ref[...].astype(f32).reshape(1, D)
        o_ref[:, 0:D] = (qb[rowblk(s - 2), :].astype(f32) * y).astype(o_ref.dtype)

    def xw(i):
        c0 = (i % 3) * D + (i // 3) * 128
        w = wstage[:, c0:c0 + 128] if lo == 1 else _unp(wq[:, c0:c0 + 128])
        r = jnp.dot(_unp(xs[...]), w, preferred_element_type=f32)
        return rungs(r, PRUNG)

    def proj_k(g):
        kc[g][_prow(base, T), :] = _pk(xw(3 * g + 1))

    def proj_q(g):
        qq = xw(3 * g) * QSCALE
        odd = (qi & DH) != 0
        qq = jnp.where(odd, jnp.concatenate([qq[HT:], qq[:HT]], axis=0), qq)
        qts[_prow(g * 128, 128), :] = _pk(qq.T)

    def proj_v(g):
        vtc[g][:, _lanes(base)] = _pk(xw(3 * g + 2).T)

    fin_old, fin_mid = lo - 2 >= 2, lo - 2 >= 1
    bres = {}

    def b_piece(j, u, mid, tok):
        bres[(j, u)] = b_exp(j, u, None if tok is None else tok[0:1], mid)
        return bres[(j, u)][2]

    if do_main:
        pieces.extend(functools.partial(conv_chain, i) for i in range(3 * 4 * T // CROWS))
    if do_fin and do_main:
        for i in range(4 * NDEF):
            pieces.insert(DSTR * i, functools.partial(b_piece, 8 - NDEF + i // 4, i % 4, fin_mid))
    if do_front and do_main and lo > 1:
        for i in range(8):
            pieces.insert(KVPOS + KVSTR * i, functools.partial(kv_piece, i))

    def wwait(g):
        slabs = [g, 4 + g, 8 + g] if g < 4 else [12, 13, 14, 15]
        for i in ([3 * g, 3 * g + 1, 3 * g + 2] if g < 4 else [12]):
            wcopy(i).wait()
        for n, i in enumerate(slabs):
            pieces.insert(2 * n, functools.partial(repack, i))
        if g == 4:
            for i in FRONT:
                cin(i, 1).wait()
            for i in FRONT:
                cin(i, 2).start()
            for i in range(8):
                pieces.insert(1 + 2 * i, functools.partial(kv_piece, i))

    if not do_main:
        if do_front:
            front_h(0)
            for i in range(8):
                kv_piece(i, None)
            front_u()
            front_h(1)
            wstart(2)
            wstart(3)
            for i in FRONT:
                cin(i, 1).start()
            wcopy(12).start()
            csmall(2).start()
            csmall(3).start()
        else:
            conv_finish()
            for j in range(8 - NDEF, 8):
                for u in range(4):
                    p, l, _ = b_exp(j, u, None, True)
                    b_pv(j, u, p, l, b_v(j, u, base - T, True, True))
            outproj(2)
            outproj(3)
            cout(s).start()
            pltpu.make_async_copy(obuf, obuf, osem.at[0]).wait()
        return

    has_old, has_mid = lo - 1 >= 2, lo - 1 >= 1
    slab = 16 * (1 + has_old) + 32 * has_mid
    in_a = ((lax.broadcasted_iota(jnp.int32, (16, T), 1) < HT)
            != (lax.broadcasted_iota(jnp.int32, (16, T), 0) >= 8))

    def blockdiag(keep, g, rows, first, n):
        ws = []
        for i in range(n):
            r0 = (first + i) * rows
            parts = []
            if r0 > 0:
                parts.append(jnp.zeros((r0, T), bf16))
            words = qts[_prow(g * 128 + r0, rows), :]
            if keep is not None:
                words = jnp.where(keep, words, jnp.zeros_like(words))
            parts.append(_unp(words))
            if r0 + rows < 128:
                parts.append(jnp.zeros((128 - r0 - rows, T), bf16))
            ws.append(jnp.concatenate(parts, axis=0))
        return jnp.concatenate(ws, axis=1)

    def stage_p(g):
        if has_old:
            sa = jnp.dot(_unp(kc[g][_prow(base - 2 * T, HT), :]), blockdiag(in_a, g, 32, 0, 4),
                         preferred_element_type=f32)
            pk[g % 2, 0:HT, :] = rungs(sa, [0])
        sbb = jnp.dot(_unp(kc[g][_prow(base + HT, HT), :]), blockdiag(~in_a, g, 32, 0, 4),
                      preferred_element_type=f32)
        pk[g % 2, HT:T, :] = rungs(sbb, [0])

    def stage_a(j):
        g = j // 2
        if 0 < j <= 8 - NDEF:
            for u in range(4):
                pieces.insert(BPOS + BSTR * u, functools.partial(b_piece, j - 1, u, has_mid))
        w = blockdiag(None, g, 16, (j % 2) * 4, 4)
        lhs = []
        for p in range(4):
            lhs.append(kc[g][_prow(base + p * 16, 16), :])
            if has_old:
                lhs.append(kc[g][_prow(base - 2 * T + HT + p * 16, 16), :])
            if has_mid:
                lhs.append(kc[g][_prow(base - T + p * 32, 32), :])
        lhs = _unp(jnp.concatenate(lhs, axis=0))
        sc = jnp.dot(lhs, w, preferred_element_type=f32)
        for u in range(4):
            su = sc[:, u * 128:(u + 1) * 128]
            tri = tris[u % 2]
            pl_ = slice(((j % 2) * 2 + u // 2) * 128, ((j % 2) * 2 + u // 2 + 1) * 128)
            mm = None
            for p in range(4):
                b0 = p * slab
                r0 = p * 16
                lo_ = jnp.where(tri[r0:r0 + 16], su[b0:b0 + 16], pk[g % 2, r0:r0 + 16, pl_] if has_old else NEG)
                hi_ = jnp.where(tri[HT + r0:HT + r0 + 16], pk[g % 2, HT + r0:HT + r0 + 16, pl_],
                                su[b0 + 16:b0 + 32] if has_old else NEG)
                if u == 0:
                    lo_ = jnp.concatenate([rung(lo_[:8]), lo_[8:]], axis=0)
                    if has_old:
                        hi_ = jnp.concatenate([rung(hi_[:8]), hi_[8:]], axis=0)
                sb[j % 2][u, r0:r0 + 16, :] = lo_
                sb[j % 2][u, HT + r0:HT + r0 + 16, :] = hi_
                c8 = jnp.maximum(jnp.maximum(lo_[:8], lo_[8:]), jnp.maximum(hi_[:8], hi_[8:]))
                mm = c8 if mm is None else jnp.maximum(mm, c8)
                if has_mid:
                    mid = su[b0 + slab - 32:b0 + slab]
                    sb[j % 2][u, T + p * 32:T + (p + 1) * 32, :] = mid
                    mm = jnp.maximum(mm, mid.reshape(4, 8, T).max(axis=0))
            mb[j % 2][u] = jnp.broadcast_to(jnp.max(mm, axis=0, keepdims=True), (8, T))

    def stage_pv(j):
        for pc in [pc for pc in pieces if pc.func is b_piece and pc.args[0] == j]:
            pieces.remove(pc)
            pc(None)
        for u in range(4):
            p, l, _ = bres.pop((j, u))
            b_pv(j, u, p, l, vdef[(j, u)] if (j, u) in vdef else b_v(j, u, base, has_old, has_mid))

    xs[...] = pltpu.bitcast(xb[rowblk(t), :], u32)
    vdef = {}
    if do_fin:
        vdef = {(j, u): b_v(j, u, base - T, fin_old, fin_mid) for j in range(8 - NDEF, 8) for u in range(4)}
    ops = dict(K=proj_k, Q=proj_q, V=proj_v, P=stage_p, A=stage_a, B=stage_pv, O=outproj, w=wwait)
    seen_a0 = False
    for op in (ORDER1 if lo == 1 else ORDER if lo + LA < NB else ORDER2).split():
        if op == 'A0':
            seen_a0 = True
        if op == 'inv' or (op[0] in 'BO' and not seen_a0) or op == 'O3':
            if do_fin:
                conv_finish() if op == 'inv' else ops[op[0]](int(op[1]))
        elif op in ('Hf', 'Uf'):
            if op == 'Hf':
                for c in front_hs():
                    front_h(c)
            elif do_front:
                front_u()
        else:
            ops[op[0]](int(op[1]))
    while pieces:
        pieces.pop(0)(None)
    if do_fin:
        cout(s).start()


def _kernel(*refs):
    for lo, hi in VARIANTS:
        if lo == hi:
            _step(lo, hi, lo, *refs)
        else:
            def body(s, c, lo=lo, hi=hi):
                _step(lo, hi, jnp.minimum(jnp.maximum(s, lo), hi), *refs)
                return c
            lax.fori_loop(lo, hi + 1, body, 0)


_FWD, _INV = (_pack_np(a) for a in _dft_consts())


@jax.jit
def pallas_concat_heads__ssm_conv_h3__sliding_block__prompt_kernel(A_q, A_k, A_v, A_shift_k, A_ssm_k, A_ssm_D, B_x, B_wqkv, B_wo):
    return pl.pallas_call(
        _kernel,
        in_specs=[pl.BlockSpec(memory_space=pl.ANY)] * 11,
        out_specs=pl.BlockSpec(memory_space=pl.ANY),
        out_shape=jax.ShapeDtypeStruct((1, S, 2 * D), bf16),
        scratch_shapes=[
            pltpu.VMEM((S, D), bf16), pltpu.VMEM((S, D), bf16),
            pltpu.VMEM((S, D), bf16), pltpu.VMEM((S, D), bf16),
            pltpu.VMEM((D, S), bf16),
            pltpu.VMEM((4, D), bf16),
            pltpu.VMEM((D,), bf16),
            pltpu.VMEM((T, T), u32),
            pltpu.VMEM((T // 2, 2 * T), u32),
            pltpu.VMEM((S, 2 * D), bf16),
            pltpu.SemaphoreType.DMA((9,)),
            pltpu.SemaphoreType.DMA((1,)),
            pltpu.VMEM((D, 4 * D), bf16),
            pltpu.VMEM((D // 2, 3 * D), u32),
            pltpu.VMEM((D // 2, D), u32),
            pltpu.SemaphoreType.DMA((13,)),
            pltpu.VMEM((T // 2, D), u32),
        ] + [pltpu.VMEM((S // 2, 128), u32)] * 4
          + [pltpu.VMEM((64, S), u32)] * 4 + [
            pltpu.VMEM((4, 2 * T, T), f32), pltpu.VMEM((4, 2 * T, T), f32),
            pltpu.VMEM((4, 8, T), f32), pltpu.VMEM((4, 8, T), f32),
            pltpu.VMEM((2, T, 4 * T), f32),
            pltpu.VMEM((NB + LA, 3, T, D), f32),
            pltpu.VMEM((NB, 3, T, D), f32),
            pltpu.VMEM((2 * T, D), f32),
            pltpu.VMEM((8, D), f32),
            pltpu.VMEM((T, D), u32),
            pltpu.VMEM((D // 2, T), u32),
            pltpu.VMEM((4, T // 2, D), u32),
            pltpu.VMEM((D, T), f32),
            pltpu.VMEM((T, D), f32),
        ],
        compiler_params=pltpu.CompilerParams(vmem_limit_bytes=100 * 1024 * 1024),
    )(A_q, A_k, A_v, A_shift_k.T, A_ssm_k, A_ssm_D, B_x, B_wqkv, B_wo,
      jnp.asarray(_FWD), jnp.asarray(_INV))
```
